```python
import jax
import jax.numpy as jnp

def _softmax(x, axis=-1):
    return jax.nn.softmax(x, axis=axis)
def _gelu(x):
    return jax.nn.gelu(x, approximate=True)
def _silu(x):
    return jax.nn.silu(x)
def _sigmoid(x):
    return jax.nn.sigmoid(x)
def _layernorm(x, axis=-1, eps=1e-5):
    m = jnp.mean(x, axis=axis, keepdims=True)
    v = jnp.var(x, axis=axis, keepdims=True)
    return (x - m) / jnp.sqrt(v + eps)
def _scatter_add(tgt, idx, src, axis=0):
    return tgt.at[idx].add(src)
def _segment_sum(src, seg, n):
    return jax.ops.segment_sum(src, seg, n)
class _Rng:
    def __init__(self, key):
        self._k = key
    def _next(self):
        self._k, sub = jax.random.split(self._k)
        return sub
    def normal(self, shape):
        return jax.random.normal(self._next(), shape, dtype=jnp.bfloat16)
    def randint(self, lo, hi, shape):
        return jax.random.randint(self._next(), shape, lo, hi, dtype=jnp.int32)
    def uniform(self, shape, lo=0.0, hi=1.0):
        return jax.random.uniform(self._next(), shape, jnp.bfloat16, lo, hi)
    def permutation(self, n):
        return jax.random.permutation(self._next(), n)


kernel_name = 'concat_heads__mha_block_cached__compressed_kv_cla__decode'

def setup_inputs():
    _rng = _Rng(jax.random.key(int.from_bytes(__import__("os").urandom(4), "little")))
    _w = (lambda a: (lambda t: t.astype(jnp.bfloat16) if jnp.issubdtype(t.dtype, jnp.floating) else t)(jnp.asarray(a)))
    def _A_setup():
        B, Sq, D = 4, 1, 576
        H, Sk, Dh = 32, 4096, 128
        return {
            "x": _w((lambda *s: _rng.normal(s) * 0.05)(B, Sq, D)),
            "k_cache": _w((lambda *s: _rng.normal(s) * 0.05)(B, H, Sk, Dh)),
            "v_cache": _w((lambda *s: _rng.normal(s) * 0.05)(B, H, Sk, Dh)),
            "wq": _w((lambda *s: _rng.normal(s) * 0.05)(D, H * Dh) * (D ** -0.5)),
            "wo": _w((lambda *s: _rng.normal(s) * 0.05)(H * Dh, D) * ((H * Dh) ** -0.5)),
        }
    _A_in = _A_setup()

    def _B_setup():
        B, H, Sq, Sk, D, M = 4, 32, 1, 4096, 128, 576
        Dc = 4 * D
        return {
            "x": _w((lambda *s: _rng.normal(s) * 0.05)(B, Sq, M)),
            "c_kv": _w((lambda *s: _rng.normal(s) * 0.05)(B, Sk, Dc)),
            "w_q": _w((lambda *s: _rng.normal(s) * 0.05)(M, H, D) * (M ** -0.5)),
            "w_uk": _w((lambda *s: _rng.normal(s) * 0.05)(Dc, H, D) * (Dc ** -0.5)),
            "w_uv": _w((lambda *s: _rng.normal(s) * 0.05)(Dc, H, D) * (Dc ** -0.5)),
            "w_o": _w((lambda *s: _rng.normal(s) * 0.05)(H, D, M) * ((H * D) ** -0.5)),
        }
    _B_in = _B_setup()

    return {
        "A_x": _A_in["x"],
        "A_k_cache": _A_in["k_cache"],
        "A_v_cache": _A_in["v_cache"],
        "A_wq": _A_in["wq"],
        "A_wo": _A_in["wo"],
        "B_x": _B_in["x"],
        "B_c_kv": _B_in["c_kv"],
        "B_w_q": _B_in["w_q"],
        "B_w_uk": _B_in["w_uk"],
        "B_w_uv": _B_in["w_uv"],
        "B_w_o": _B_in["w_o"],
    }

def reference(A_x, A_k_cache, A_v_cache, A_wq, A_wo, B_x, B_c_kv, B_w_q, B_w_uk, B_w_uv, B_w_o):
    def _A_ref(x, k_cache, v_cache, wq, wo):
        B, Sq, D = x.shape
        H, Dh = 32, 128
        q = (lambda x, *d: x.transpose(*d))((x @ wq).reshape(B, Sq, H, Dh), 0, 2, 1, 3)
        scores = jnp.einsum("bhqd,bhkd->bhqk", q, k_cache) * (Dh ** -0.5)
        p = _softmax(scores, axis=-1)
        o = jnp.einsum("bhqk,bhkd->bhqd", p, v_cache)
        return (lambda x, *d: x.transpose(*d))(o, 0, 2, 1, 3).reshape(B, Sq, H * Dh) @ wo

    def _B_ref(x, c_kv, w_q, w_uk, w_uv, w_o):
        B, Sq, M = x.shape[0], x.shape[1], x.shape[2]
        Sk = c_kv.shape[1]
        H, D = w_q.shape[1], w_q.shape[2]
        q = jnp.einsum("bqm,mhd->bhqd", x, w_q)
        k = jnp.einsum("bkc,chd->bhkd", c_kv, w_uk)
        v = jnp.einsum("bkc,chd->bhkd", c_kv, w_uv)
        scores = jnp.einsum("bhqd,bhkd->bhqk", q, k) * (D ** -0.5)
        off = Sk - Sq
        qi = jnp.arange(Sq)[:, None]
        kj = jnp.arange(Sk)[None, :]
        cmask = kj <= (qi + off)
        scores = jnp.where(cmask[None, None], scores, -1e9)
        p = _softmax(scores, axis=-1)
        ctx = jnp.einsum("bhqk,bhkd->bhqd", p, v)
        return jnp.einsum("bhqd,hdm->bqm", ctx, w_o)

    a = _A_ref(A_x, A_k_cache, A_v_cache, A_wq, A_wo)
    b = _B_ref(B_x, B_c_kv, B_w_q, B_w_uk, B_w_uv, B_w_o)
    return jnp.concatenate([a, b], axis=-1)
```

```python
import jax
import jax.numpy as jnp
import jax.experimental.pallas as pl
import jax.experimental.pallas.tpu as pltpu

B = 4
H = 32
SK = 4096
DH = 128
DM = 576
DC = 512
HD = H * DH

NSLOT = 6
KV_ROWS = 128
KV_CH = SK // KV_ROWS

F32 = jnp.float32
BF16 = jnp.bfloat16


def _softmax_rows(s):
    m = jnp.max(s, axis=-1, keepdims=True)
    p = jnp.exp(s - m)
    l = jnp.sum(p, axis=-1, keepdims=True)
    return p, l


def _kernel(xa_hbm, k_hbm, v_hbm, wq_hbm, wo_hbm,
            xb_hbm, ckv_hbm, wqb_hbm, wuk_hbm, wuv_hbm, wob_hbm,
            o_ref,
            xa_v, xb_v, wq_v, wo_v, wqb_v, wuk_v, wuv_v, wob_v, ckv_v,
            kbuf, vbuf, qa_s, oa_s, ctxc_s,
            wsem, kvsem):
    SEM_XA, SEM_XB, SEM_WQ, SEM_WO, SEM_WQB, SEM_WUK, SEM_WUV, SEM_WOB = range(8)
    SEM_CKV = 8

    def wait_all(buf, sem):
        pltpu.make_async_copy(buf, buf, sem).wait()

    def start_kv(b, h, slot):
        for g in range(KV_CH):
            rows = pl.ds(g * KV_ROWS, KV_ROWS)
            pltpu.make_async_copy(k_hbm.at[b, h, rows, :], kbuf.at[slot, rows, :],
                                  kvsem.at[0, slot]).start(priority=0)
            pltpu.make_async_copy(v_hbm.at[b, h, rows, :], vbuf.at[slot, rows, :],
                                  kvsem.at[1, slot]).start(priority=1)

    def issue_loop(n, fn):
        def body(i, c):
            fn(i)
            return c
        lax_fori(0, n, body)

    def lax_fori(lo, hi, body):
        jax.lax.fori_loop(lo, hi, body, 0)

    pltpu.make_async_copy(xa_hbm, xa_v, wsem.at[SEM_XA]).start(priority=0)
    pltpu.make_async_copy(xb_hbm, xb_v, wsem.at[SEM_XB]).start(priority=1)

    def issue_wq(i):
        r = pl.multiple_of((i // 2) * 8, 8)
        c = pl.multiple_of((i % 2) * 2048, 2048)
        pltpu.make_async_copy(wq_hbm.at[pl.ds(r, 8), pl.ds(c, 2048)],
                              wq_v.at[pl.ds(r, 8), pl.ds(c, 2048)],
                              wsem.at[SEM_WQ]).start(priority=0)
        pltpu.make_async_copy(wqb_hbm.at[pl.ds(i * 4, 4)], wqb_v.at[pl.ds(i * 4, 4)],
                              wsem.at[SEM_WQB]).start(priority=1)
    issue_loop(144, issue_wq)

    def issue_wu(i):
        pltpu.make_async_copy(wuk_hbm.at[pl.ds(i * 4, 4)], wuk_v.at[pl.ds(i * 4, 4)],
                              wsem.at[SEM_WUK]).start(priority=0)
        pltpu.make_async_copy(wuv_hbm.at[pl.ds(i * 4, 4)], wuv_v.at[pl.ds(i * 4, 4)],
                              wsem.at[SEM_WUV]).start(priority=1)
    issue_loop(128, issue_wu)

    wait_all(xa_v, wsem.at[SEM_XA])
    wait_all(wq_v, wsem.at[SEM_WQ])
    xa = xa_v[...]
    qa = jnp.dot(xa, wq_v[...], preferred_element_type=F32).astype(BF16)
    for h in range(H):
        qa_s[h] = qa[:, h * DH:(h + 1) * DH]

    def issue_ckv(pair):
        def f(i):
            r = pl.multiple_of(i * 32, 32)
            for s in range(2):
                bb = pair + 2 * s
                pltpu.make_async_copy(ckv_hbm.at[bb, pl.ds(r, 32), :],
                                      ckv_v.at[bb, pl.ds(r, 32), :],
                                      wsem.at[SEM_CKV + bb]).start(priority=s)
        return f
    issue_loop(128, issue_ckv(0))

    wait_all(xb_v, wsem.at[SEM_XB])
    wait_all(wqb_v, wsem.at[SEM_WQB])
    xb = xb_v[...]
    qb = jnp.dot(xb, wqb_v[...].reshape(DM, HD), preferred_element_type=F32).astype(BF16)

    issue_loop(128, issue_ckv(1))

    row_h = jax.lax.broadcasted_iota(jnp.int32, (B * H, HD), 0) % H
    col_h = jax.lax.broadcasted_iota(jnp.int32, (B * H, HD), 1) // DH
    diag = row_h == col_h
    wait_all(wuk_v, wsem.at[SEM_WUK])
    qb_rows = jnp.broadcast_to(qb.astype(F32)[:, None, :], (B, H, HD)).reshape(B * H, HD)
    qblk = jnp.where(diag, qb_rows, 0.0).astype(BF16)
    qabs = jax.lax.dot_general(qblk, wuk_v[...].reshape(DC, HD), (((1,), (1,)), ((), ())),
                               preferred_element_type=F32).astype(BF16)

    def issue_wo(i):
        r = pl.multiple_of((i // 2) * 8, 8)
        c = pl.multiple_of((i % 2) * 2048, 2048)
        pltpu.make_async_copy(wo_hbm.at[pl.ds(r, 8), pl.ds(c, 2048)],
                              wo_v.at[pl.ds(r, 8), pl.ds(c, 2048)],
                              wsem.at[SEM_WO]).start(priority=0)
        rr = pl.multiple_of(i * 128, 128)
        pltpu.make_async_copy(wob_hbm.at[pl.ds(rr, 128), :], wob_v.at[pl.ds(rr, 128), :],
                              wsem.at[SEM_WOB]).start(priority=1)
    issue_loop(144, issue_wo)

    for t in range(NSLOT):
        start_kv(t % B, t // B, t)

    for b in (0, 2, 1, 3):
        wait_all(ckv_v.at[b], wsem.at[SEM_CKV + b])
        c = ckv_v[b]
        s = jax.lax.dot_general(qabs[b * H:(b + 1) * H], c, (((1,), (1,)), ((), ())),
                                preferred_element_type=F32) * (DH ** -0.5)
        p, l = _softmax_rows(s)
        cc = jnp.dot(p.astype(BF16), c, preferred_element_type=F32) / l
        ctxc_s[b * H:(b + 1) * H, :] = cc.astype(BF16)

    wait_all(wuv_v, wsem.at[SEM_WUV])
    ctx_all = jnp.dot(ctxc_s[...], wuv_v[...].reshape(DC, HD), preferred_element_type=F32)
    ctx = jnp.sum(jnp.where(diag, ctx_all, 0.0).reshape(B, H, HD), axis=1).astype(BF16)
    wait_all(wob_v, wsem.at[SEM_WOB])
    out_b = jnp.zeros((B, DM), F32)
    for h in range(H):
        out_b = out_b + jax.lax.dot_general(
            ctx[:, h * DH:(h + 1) * DH], wob_v[h * DM:(h + 1) * DM, :],
            (((1,), (1,)), ((), ())), preferred_element_type=F32)

    wait_all(wo_v, wsem.at[SEM_WO])

    row4 = jax.lax.broadcasted_iota(jnp.int32, (B, DH), 0)

    def head_body(h, carry):
        q = qa_s[h]
        o_h = jnp.zeros((B, DH), F32)
        for b in range(B):
            t = h * B + b
            slot = t % NSLOT
            wait_all(kbuf.at[slot], kvsem.at[0, slot])
            s = jax.lax.dot_general(q, kbuf[slot], (((1,), (1,)), ((), ())),
                                    preferred_element_type=F32) * (DH ** -0.5)
            p, l = _softmax_rows(s)
            wait_all(vbuf.at[slot], kvsem.at[1, slot])
            o = jnp.dot(p.astype(BF16), vbuf[slot], preferred_element_type=F32) / l
            o_h = jnp.where(row4 == b, o, o_h)

            tn = t + NSLOT

            @pl.when(tn < H * B)
            def _():
                start_kv(tn % B, tn // B, slot)

        oa_s[h] = o_h
        return carry

    jax.lax.fori_loop(0, H, head_body, 0)

    oa = jnp.concatenate([oa_s[h] for h in range(H)], axis=-1).astype(BF16)
    out_a = jax.lax.dot_general(oa, wo_v[...], (((1,), (1,)), ((), ())),
                                preferred_element_type=F32)
    o_ref[...] = jnp.concatenate([out_a, out_b], axis=-1).astype(BF16)


@jax.jit
def pallas_concat_heads__mha_block_cached__compressed_kv_cla__decode_kernel(
    A_x: jax.Array,
    A_k_cache: jax.Array,
    A_v_cache: jax.Array,
    A_wq: jax.Array,
    A_wo: jax.Array,
    B_x: jax.Array,
    B_c_kv: jax.Array,
    B_w_q: jax.Array,
    B_w_uk: jax.Array,
    B_w_uv: jax.Array,
    B_w_o: jax.Array,
):
    hbm = pl.BlockSpec(memory_space=pl.ANY)
    xa = A_x.reshape(B, DM)
    xb = B_x.reshape(B, DM)
    wo_t = A_wo.T
    wob_t = jnp.transpose(B_w_o, (0, 2, 1)).reshape(H * DM, DH)
    out = pl.pallas_call(
        _kernel,
        in_specs=[hbm] * 11,
        out_specs=pl.BlockSpec(memory_space=pltpu.VMEM),
        out_shape=jax.ShapeDtypeStruct((B, 2 * DM), BF16),
        scratch_shapes=[
            pltpu.VMEM((B, DM), BF16),
            pltpu.VMEM((B, DM), BF16),
            pltpu.VMEM((DM, HD), BF16),
            pltpu.VMEM((DM, HD), BF16),
            pltpu.VMEM((DM, H, DH), BF16),
            pltpu.VMEM((DC, H, DH), BF16),
            pltpu.VMEM((DC, H, DH), BF16),
            pltpu.VMEM((H * DM, DH), BF16),
            pltpu.VMEM((B, SK, DC), BF16),
            pltpu.VMEM((NSLOT, SK, DH), BF16),
            pltpu.VMEM((NSLOT, SK, DH), BF16),
            pltpu.VMEM((H, B, DH), BF16),
            pltpu.VMEM((H, B, DH), F32),
            pltpu.VMEM((B * H, DC), BF16),
            pltpu.SemaphoreType.DMA((8 + B,)),
            pltpu.SemaphoreType.DMA((2, NSLOT)),
        ],
        compiler_params=pltpu.CompilerParams(vmem_limit_bytes=110 * 1024 * 1024),
    )(xa, A_k_cache, A_v_cache, A_wq, wo_t, xb, B_c_kv, B_w_q, B_w_uk, B_w_uv, wob_t)
    return out.reshape(B, 1, 2 * DM)
```

```python
import jax
import jax.numpy as jnp
import jax.experimental.pallas as pl
import jax.experimental.pallas.tpu as pltpu

B = 4
H = 32
SK = 4096
DH = 128
DM = 576
DC = 512
HD = H * DH
NPAIR = B * H
NBLK = 2 * NPAIR

NSLOT = 8
ROWS = 128
NS = 8
CPB = SK // ROWS // NS
DELTA = 2
LOOK = 12
PRING = 8
VSPLIT = 2
HG = 8

F32 = jnp.float32
BF16 = jnp.bfloat16
NT = (((1,), (1,)), ((), ()))
SCALE = DH ** -0.5


def _softmax_rows(s):
    m = jnp.max(s, axis=-1, keepdims=True)
    p = jnp.exp(s - m)
    l = jnp.sum(p, axis=-1, keepdims=True)
    return p, l


def _kernel(xa_hbm, k_hbm, v_hbm, wq_hbm, wo_hbm,
            xb_hbm, ckv_hbm, wqb_hbm, wuk_hbm, wuv_hbm, wob_hbm,
            o_ref,
            xa_v, xb_v, wq_v, wo_v, wqb_v, wuk_v, wuv_v, wob_v, ckv_v,
            kbuf, vbuf, qa_s, woh_s, p_s, l_s, qabs_s, pb_s, lb_s, ctxc_s,
            wsem, kvsem):
    SEM_XA, SEM_XB, SEM_WQ, SEM_WO, SEM_WQB, SEM_WUK, SEM_WUV, SEM_WOB = range(8)
    SEM_CKV = 8

    def wait_all(buf, sem):
        pltpu.make_async_copy(buf, buf, sem).wait()

    def copy(src, dst, sem, queue):
        pltpu.make_async_copy(src, dst, sem).start(priority=queue)

    def rounds(lo, hi, fn):
        def body(i, c):
            fn(i)
            return c
        jax.lax.fori_loop(lo, hi, body, 0)

    def cp_2d(src, dst, sem, i, queue):
        r = pl.multiple_of((i // 2) * 8, 8)
        c = pl.multiple_of((i % 2) * 2048, 2048)
        copy(src.at[pl.ds(r, 8), pl.ds(c, 2048)], dst.at[pl.ds(r, 8), pl.ds(c, 2048)],
             sem, queue)

    def cp_3d(src, dst, sem, i, queue):
        copy(src.at[pl.ds(i * 4, 4)], dst.at[pl.ds(i * 4, 4)], sem, queue)

    def cp_ckv(b, i, queue):
        r = pl.multiple_of(i * 32, 32)
        copy(ckv_hbm.at[b, pl.ds(r, 32), :], ckv_v.at[b, pl.ds(r, 32), :],
             wsem.at[SEM_CKV + b], queue)

    def cp_wob(i, queue):
        r = pl.multiple_of(i * 128, 128)
        copy(wob_hbm.at[pl.ds(r, 128), :], wob_v.at[pl.ds(r, 128), :],
             wsem.at[SEM_WOB], queue)

    def pa_round(i):
        for quarter in range(4):
            cp_3d(wqb_hbm, wqb_v, wsem.at[SEM_WQB], quarter * 36 + i, 0)
            cp_3d(wuk_hbm, wuk_v, wsem.at[SEM_WUK], quarter * 32 + i, 1)

    def pa_tail(i):
        for quarter in range(4):
            cp_3d(wqb_hbm, wqb_v, wsem.at[SEM_WQB], quarter * 36 + i, quarter % 2)

    def pc_round(b0):
        def f(i):
            for quarter in range(4):
                cp_ckv(b0, quarter * 32 + i, 0)
                cp_ckv(b0 + 1, quarter * 32 + i, 1)
        return f

    def pd_round(i):
        for quarter in range(4):
            cp_wob(quarter * 36 + i, 0)
            cp_3d(wuv_hbm, wuv_v, wsem.at[SEM_WUV], quarter * 32 + i, 1)

    def pd_tail(i):
        for quarter in range(4):
            cp_wob(quarter * 36 + i, quarter % 2)

    def p2d_round(src, dst, sem):
        def f(i):
            for s8 in range(8):
                cp_2d(src, dst, sem, s8 * 18 + i, s8 % 2)
        return f

    def kv_step(j, parity, only=None):
        static = isinstance(j, int)
        blocks = []
        for i in range(NS):
            isv = (parity - i) % 2
            t = (j - i - isv) // 2
            if (static and not (0 <= j - i < NBLK)) or (only is not None and isv != only):
                blocks.append(None)
                continue
            blocks.append((isv, t % B, t // B, t % NSLOT))
        for c in range(CPB):
            for i in range(NS):
                if blocks[i] is None:
                    continue
                isv, b, h, slot = blocks[i]
                rows = pl.ds((i * CPB + c) * ROWS, ROWS)
                src, dst = (v_hbm, vbuf) if isv else (k_hbm, kbuf)
                copy(src.at[b, h, rows, :], dst.at[slot, rows, :],
                     kvsem.at[isv, slot], isv)

    def group_mask():
        r = jax.lax.broadcasted_iota(jnp.int32, (B * HG, HG * DH), 0) % HG
        c = jax.lax.broadcasted_iota(jnp.int32, (B * HG, HG * DH), 1) // DH
        return r == c

    def b_query(g):
        hs = slice(g * HG, (g + 1) * HG)
        qg = jnp.dot(xb_v[...], wqb_v[:, hs, :].reshape(DM, HG * DH),
                     preferred_element_type=F32).astype(BF16).astype(F32)
        rows = jnp.broadcast_to(qg[:, None, :], (B, HG, HG * DH)).reshape(B * HG, HG * DH)
        qblk = jnp.where(group_mask(), rows, 0.0).astype(BF16)
        qa = jax.lax.dot_general(qblk, wuk_v[:, hs, :].reshape(DC, HG * DH), NT,
                                 preferred_element_type=F32)
        for b in range(B):
            qabs_s[b * H + g * HG:b * H + (g + 1) * HG, :] = qa[b * HG:(b + 1) * HG]

    def b_scores(b):
        q = qabs_s[b * H:(b + 1) * H, :].astype(BF16)
        s = jax.lax.dot_general(q, ckv_v[b], NT, preferred_element_type=F32) * SCALE
        p, l = _softmax_rows(s)
        pb_s[...] = p.astype(BF16)
        lb_s[...] = jnp.broadcast_to(l, lb_s.shape)

    def b_values(b):
        cc = jnp.dot(pb_s[...], ckv_v[b], preferred_element_type=F32)
        ctxc_s[b * H:(b + 1) * H, :] = cc / lb_s[:, 0:1]

    def b_out(g, acc):
        hs = slice(g * HG, (g + 1) * HG)
        lhs = jnp.concatenate(
            [ctxc_s[b * H + g * HG:b * H + (g + 1) * HG, :] for b in range(B)],
            axis=0).astype(BF16)
        full = jnp.dot(lhs, wuv_v[:, hs, :].reshape(DC, HG * DH),
                       preferred_element_type=F32)
        ctx = jnp.sum(jnp.where(group_mask(), full, 0.0).reshape(B, HG, HG * DH),
                      axis=1).astype(BF16)
        for j in range(HG):
            h = g * HG + j
            acc = acc + jax.lax.dot_general(
                ctx[:, j * DH:(j + 1) * DH], wob_v[h * DM:(h + 1) * DM, :], NT,
                preferred_element_type=F32)
        return acc

    def w_wait(buf, idx):
        wait_all(buf, wsem.at[idx])

    copy(xb_hbm, xb_v, wsem.at[SEM_XB], 0)
    copy(xa_hbm, xa_v, wsem.at[SEM_XA], 1)
    rounds(0, 32, pa_round)
    rounds(32, 36, pa_tail)
    rounds(0, 15, pc_round(0))
    w_wait(xb_v, SEM_XB)
    w_wait(wqb_v, SEM_WQB)
    w_wait(wuk_v, SEM_WUK)
    b_query(0)
    rounds(15, 20, pc_round(0))
    b_query(1)
    rounds(20, 26, pc_round(0))
    b_query(2)
    rounds(26, 32, pc_round(0))
    b_query(3)
    rounds(0, 8, pc_round(2))
    w_wait(ckv_v.at[0], SEM_CKV + 0)
    b_scores(0)
    rounds(8, 14, pc_round(2))
    b_values(0)
    rounds(14, 18, pc_round(2))
    w_wait(ckv_v.at[1], SEM_CKV + 1)
    b_scores(1)
    rounds(18, 24, pc_round(2))
    b_values(1)
    rounds(24, 32, pc_round(2))
    rounds(0, 8, pd_round)
    w_wait(ckv_v.at[2], SEM_CKV + 2)
    b_scores(2)
    rounds(8, 14, pd_round)
    b_values(2)
    rounds(14, 18, pd_round)
    w_wait(ckv_v.at[3], SEM_CKV + 3)
    b_scores(3)
    rounds(18, 24, pd_round)
    b_values(3)
    rounds(24, 32, pd_round)
    rounds(32, 36, pd_tail)
    wo_round = p2d_round(wo_hbm, wo_v, wsem.at[SEM_WO])
    wq_round = p2d_round(wq_hbm, wq_v, wsem.at[SEM_WQ])
    rounds(0, 14, wo_round)
    w_wait(wuv_v, SEM_WUV)
    w_wait(wob_v, SEM_WOB)
    out_b = jnp.zeros((B, DM), F32)
    out_b = b_out(0, out_b)
    rounds(14, 18, wo_round)
    out_b = b_out(1, out_b)
    rounds(0, 4, wq_round)
    out_b = b_out(2, out_b)
    rounds(4, 8, wq_round)
    out_b = b_out(3, out_b)
    o_ref[:, DM:] = out_b.astype(BF16)
    rounds(8, 13, wq_round)
    w_wait(wo_v, SEM_WO)
    for h in range(H // 2):
        woh_s[h] = wo_v[:, h * DH:(h + 1) * DH]
    rounds(13, 18, wq_round)
    for h in range(H // 2, H):
        woh_s[h] = wo_v[:, h * DH:(h + 1) * DH]
    for j in range(LOOK - 2 * DELTA):
        kv_step(j, j % 2)

    w_wait(xa_v, SEM_XA)
    w_wait(wq_v, SEM_WQ)
    qa = jnp.dot(xa_v[...], wq_v[...], preferred_element_type=F32).astype(BF16)
    for h in range(H):
        qa_s[h] = qa[:, h * DH:(h + 1) * DH]

    row4 = jax.lax.broadcasted_iota(jnp.int32, (B, DH), 0)

    def scores(t):
        slot = t % NSLOT
        wait_all(kbuf.at[slot], kvsem.at[0, slot])
        s = jax.lax.dot_general(qa_s[t // B], kbuf[slot], NT,
                                preferred_element_type=F32) * SCALE
        p, l = _softmax_rows(s)
        p_s[t % PRING] = p.astype(BF16)
        l_s[t % PRING] = jnp.broadcast_to(l, (B, DH))

    def values(t, acc):
        slot = t % NSLOT
        wait_all(vbuf.at[slot], kvsem.at[1, slot])
        o = jnp.dot(p_s[t % PRING], vbuf[slot], preferred_element_type=F32) / l_s[t % PRING]
        o = jnp.where(row4 == t % B, o, 0.0).astype(BF16)
        return acc + jax.lax.dot_general(o, woh_s[t // B], NT, preferred_element_type=F32)

    def foreach(lo, hi, fn):
        def body(t, c):
            fn(t)
            return c
        jax.lax.fori_loop(lo, hi, body, 0)

    def steady(t, acc):
        kv_step(2 * t + LOOK, LOOK % 2)
        scores(t + DELTA)
        kv_step(2 * t + 1 + LOOK, (LOOK + 1) % 2)
        return jax.lax.cond(t >= 0, lambda: values(t, acc), lambda: acc)

    t_main = (NBLK - LOOK) // 2
    out_a = jax.lax.fori_loop(-DELTA, t_main, steady, jnp.zeros((B, DM), F32))
    tail_steps = range(2 * t_main + LOOK, NBLK + NS - 1)
    for j in tail_steps:
        kv_step(j, j % 2, 0)
    for j in tail_steps[:VSPLIT]:
        kv_step(j, j % 2, 1)
    out_a = values(t_main, out_a)

    def tail_scores(t):
        scores(t)

        @pl.when(t == t_main + DELTA)
        def _():
            for j in tail_steps[VSPLIT:]:
                kv_step(j, j % 2, 1)

    foreach(t_main + DELTA, NPAIR, tail_scores)
    out_a = jax.lax.fori_loop(t_main + 1, NPAIR, values, out_a)
    o_ref[:, :DM] = out_a.astype(BF16)


@jax.jit
def pallas_concat_heads__mha_block_cached__compressed_kv_cla__decode_kernel(
    A_x: jax.Array,
    A_k_cache: jax.Array,
    A_v_cache: jax.Array,
    A_wq: jax.Array,
    A_wo: jax.Array,
    B_x: jax.Array,
    B_c_kv: jax.Array,
    B_w_q: jax.Array,
    B_w_uk: jax.Array,
    B_w_uv: jax.Array,
    B_w_o: jax.Array,
):
    hbm = pl.BlockSpec(memory_space=pl.ANY)
    xa = A_x.reshape(B, DM)
    xb = B_x.reshape(B, DM)
    wo_t = A_wo.T
    wob_t = jnp.transpose(B_w_o, (0, 2, 1)).reshape(H * DM, DH)
    out = pl.pallas_call(
        _kernel,
        in_specs=[hbm] * 11,
        out_specs=pl.BlockSpec(memory_space=pltpu.VMEM),
        out_shape=jax.ShapeDtypeStruct((B, 2 * DM), BF16),
        scratch_shapes=[
            pltpu.VMEM((B, DM), BF16),
            pltpu.VMEM((B, DM), BF16),
            pltpu.VMEM((DM, HD), BF16),
            pltpu.VMEM((DM, HD), BF16),
            pltpu.VMEM((DM, H, DH), BF16),
            pltpu.VMEM((DC, H, DH), BF16),
            pltpu.VMEM((DC, H, DH), BF16),
            pltpu.VMEM((H * DM, DH), BF16),
            pltpu.VMEM((B, SK, DC), BF16),
            pltpu.VMEM((NSLOT, SK, DH), BF16),
            pltpu.VMEM((NSLOT, SK, DH), BF16),
            pltpu.VMEM((H, B, DH), BF16),
            pltpu.VMEM((H, DM, DH), BF16),
            pltpu.VMEM((PRING, B, SK), BF16),
            pltpu.VMEM((PRING, B, DH), F32),
            pltpu.VMEM((B * H, DC), F32),
            pltpu.VMEM((H, SK), BF16),
            pltpu.VMEM((H, DH), F32),
            pltpu.VMEM((B * H, DC), F32),
            pltpu.SemaphoreType.DMA((8 + B,)),
            pltpu.SemaphoreType.DMA((2, NSLOT)),
        ],
        compiler_params=pltpu.CompilerParams(vmem_limit_bytes=110 * 1024 * 1024,
                                             disable_bounds_checks=True,
                                             disable_semaphore_checks=True),
    )(xa, A_k_cache, A_v_cache, A_wq, wo_t, xb, B_c_kv, B_w_q, B_w_uk, B_w_uv, wob_t)
    return out.reshape(B, 1, 2 * DM)
```

```python
import jax
import jax.numpy as jnp
import jax.experimental.pallas as pl
import jax.experimental.pallas.tpu as pltpu

B = 4
H = 32
SK = 4096
DH = 128
DM = 576
DC = 512
HD = H * DH
NPAIR = B * H
NBLK = 2 * NPAIR

NSLOT = 8
ROWS = 128
NS = 8
CPB = SK // ROWS // NS
DELTA = 2
LOOK = 12
PRING = 8
VSPLIT = 2
HG = 8

F32 = jnp.float32
BF16 = jnp.bfloat16
NT = (((1,), (1,)), ((), ()))
SCALE = DH ** -0.5


def _softmax_rows(s):
    m = jnp.max(s, axis=-1, keepdims=True)
    p = jnp.exp(s - m)
    l = jnp.sum(p, axis=-1, keepdims=True)
    return p, l


def _kernel(xa_hbm, k_hbm, v_hbm, wq_hbm, wo_hbm,
            xb_hbm, ckv_hbm, wqb_hbm, wuk_hbm, wuv_hbm, wob_hbm,
            o_ref,
            xa_v, xb_v, wq_v, wo_v, wqb_v, wuk_v, wuv_v, wob_v, ckv_v,
            kbuf, vbuf, qa_s, woh_s, p_s, l_s, qabs_s, pb_s, lb_s, ctxc_s,
            wsem, kvsem):
    SEM_XA, SEM_XB, SEM_WQ, SEM_WO, SEM_WQB, SEM_WUK, SEM_WUV, SEM_WOB = range(8)
    SEM_CKV = 8

    def wait_all(buf, sem):
        pltpu.make_async_copy(buf, buf, sem).wait()

    def copy(src, dst, sem, queue):
        pltpu.make_async_copy(src, dst, sem).start(priority=queue)

    def rounds(lo, hi, fn):
        def body(i, c):
            fn(i)
            return c
        jax.lax.fori_loop(lo, hi, body, 0)

    def cp_2d(src, dst, sem, i, queue):
        r = pl.multiple_of((i // 2) * 8, 8)
        c = pl.multiple_of((i % 2) * 2048, 2048)
        copy(src.at[pl.ds(r, 8), pl.ds(c, 2048)], dst.at[pl.ds(r, 8), pl.ds(c, 2048)],
             sem, queue)

    def cp_3d(src, dst, sem, i, queue):
        copy(src.at[pl.ds(i * 4, 4)], dst.at[pl.ds(i * 4, 4)], sem, queue)

    def cp_ckv(b, i, queue):
        r = pl.multiple_of(i * 32, 32)
        copy(ckv_hbm.at[b, pl.ds(r, 32), :], ckv_v.at[b, pl.ds(r, 32), :],
             wsem.at[SEM_CKV + b], queue)

    def cp_wob(i, queue):
        r = pl.multiple_of(i * 128, 128)
        copy(wob_hbm.at[pl.ds(r, 128), :], wob_v.at[pl.ds(r, 128), :],
             wsem.at[SEM_WOB], queue)

    def pa_round(i):
        for quarter in range(4):
            cp_3d(wqb_hbm, wqb_v, wsem.at[SEM_WQB], quarter * 36 + i, 0)
            cp_3d(wuk_hbm, wuk_v, wsem.at[SEM_WUK], quarter * 32 + i, 1)

    def pa_tail(i):
        for quarter in range(4):
            cp_3d(wqb_hbm, wqb_v, wsem.at[SEM_WQB], quarter * 36 + i, quarter % 2)

    def pc_round(b0):
        def f(i):
            for quarter in range(4):
                cp_ckv(b0, quarter * 32 + i, 0)
                cp_ckv(b0 + 1, quarter * 32 + i, 1)
        return f

    def pd_round(i):
        for quarter in range(4):
            cp_wob(quarter * 36 + i, 0)
            cp_3d(wuv_hbm, wuv_v, wsem.at[SEM_WUV], quarter * 32 + i, 1)

    def pd_tail(i):
        for quarter in range(4):
            cp_wob(quarter * 36 + i, quarter % 2)

    def p2d_round(src, dst, sem):
        def f(i):
            for s8 in range(8):
                cp_2d(src, dst, sem, s8 * 18 + i, s8 % 2)
        return f

    def kv_step(j, parity, only=None, tail_v=False):
        static = isinstance(j, int)
        blocks = []
        for i in range(NS):
            isv = (parity - i) % 2
            t = (j - i - isv) // 2
            if (static and not (0 <= j - i < NBLK)) or (only is not None and isv != only):
                blocks.append(None)
                continue
            blocks.append((isv, t % B, t // B, t % NSLOT))
        for c in range(CPB):
            for i in range(NS):
                if blocks[i] is None:
                    continue
                isv, b, h, slot = blocks[i]
                rows = pl.ds((i * CPB + c) * ROWS, ROWS)
                src, dst = (v_hbm, vbuf) if isv else (k_hbm, kbuf)
                queue = int(j - i == NBLK - 1) if tail_v else isv
                copy(src.at[b, h, rows, :], dst.at[slot, rows, :],
                     kvsem.at[isv, slot], queue)

    def group_mask():
        r = jax.lax.broadcasted_iota(jnp.int32, (B * HG, HG * DH), 0) % HG
        c = jax.lax.broadcasted_iota(jnp.int32, (B * HG, HG * DH), 1) // DH
        return r == c

    def b_query(g):
        hs = slice(g * HG, (g + 1) * HG)
        qg = jnp.dot(xb_v[...], wqb_v[:, hs, :].reshape(DM, HG * DH),
                     preferred_element_type=F32).astype(BF16).astype(F32)
        rows = jnp.broadcast_to(qg[:, None, :], (B, HG, HG * DH)).reshape(B * HG, HG * DH)
        qblk = jnp.where(group_mask(), rows, 0.0).astype(BF16)
        qa = jax.lax.dot_general(qblk, wuk_v[:, hs, :].reshape(DC, HG * DH), NT,
                                 preferred_element_type=F32)
        for b in range(B):
            qabs_s[b * H + g * HG:b * H + (g + 1) * HG, :] = qa[b * HG:(b + 1) * HG]

    def b_scores(b):
        q = qabs_s[b * H:(b + 1) * H, :].astype(BF16)
        s = jax.lax.dot_general(q, ckv_v[b], NT, preferred_element_type=F32) * SCALE
        p, l = _softmax_rows(s)
        pb_s[...] = p.astype(BF16)
        lb_s[...] = jnp.broadcast_to(l, lb_s.shape)

    def b_values(b):
        cc = jnp.dot(pb_s[...], ckv_v[b], preferred_element_type=F32)
        ctxc_s[b * H:(b + 1) * H, :] = cc / lb_s[:, 0:1]

    def b_out(g, acc):
        hs = slice(g * HG, (g + 1) * HG)
        lhs = jnp.concatenate(
            [ctxc_s[b * H + g * HG:b * H + (g + 1) * HG, :] for b in range(B)],
            axis=0).astype(BF16)
        full = jnp.dot(lhs, wuv_v[:, hs, :].reshape(DC, HG * DH),
                       preferred_element_type=F32)
        ctx = jnp.sum(jnp.where(group_mask(), full, 0.0).reshape(B, HG, HG * DH),
                      axis=1).astype(BF16)
        for j in range(HG):
            h = g * HG + j
            acc = acc + jax.lax.dot_general(
                ctx[:, j * DH:(j + 1) * DH], wob_v[h * DM:(h + 1) * DM, :], NT,
                preferred_element_type=F32)
        return acc

    def w_wait(buf, idx):
        wait_all(buf, wsem.at[idx])

    copy(xb_hbm, xb_v, wsem.at[SEM_XB], 0)
    copy(xa_hbm, xa_v, wsem.at[SEM_XA], 1)
    rounds(0, 32, pa_round)
    rounds(32, 36, pa_tail)
    rounds(0, 15, pc_round(0))
    w_wait(xb_v, SEM_XB)
    w_wait(wqb_v, SEM_WQB)
    w_wait(wuk_v, SEM_WUK)
    b_query(0)
    rounds(15, 20, pc_round(0))
    b_query(1)
    rounds(20, 26, pc_round(0))
    b_query(2)
    rounds(26, 32, pc_round(0))
    b_query(3)
    rounds(0, 8, pc_round(2))
    w_wait(ckv_v.at[0], SEM_CKV + 0)
    b_scores(0)
    rounds(8, 14, pc_round(2))
    b_values(0)
    rounds(14, 18, pc_round(2))
    w_wait(ckv_v.at[1], SEM_CKV + 1)
    b_scores(1)
    rounds(18, 24, pc_round(2))
    b_values(1)
    rounds(24, 32, pc_round(2))
    rounds(0, 8, pd_round)
    w_wait(ckv_v.at[2], SEM_CKV + 2)
    b_scores(2)
    rounds(8, 14, pd_round)
    b_values(2)
    rounds(14, 18, pd_round)
    w_wait(ckv_v.at[3], SEM_CKV + 3)
    b_scores(3)
    rounds(18, 24, pd_round)
    b_values(3)
    rounds(24, 32, pd_round)
    rounds(32, 36, pd_tail)
    wo_round = p2d_round(wo_hbm, wo_v, wsem.at[SEM_WO])
    wq_round = p2d_round(wq_hbm, wq_v, wsem.at[SEM_WQ])
    rounds(0, 14, wo_round)
    w_wait(wuv_v, SEM_WUV)
    w_wait(wob_v, SEM_WOB)
    out_b = jnp.zeros((B, DM), F32)
    out_b = b_out(0, out_b)
    rounds(14, 18, wo_round)
    out_b = b_out(1, out_b)
    rounds(0, 4, wq_round)
    out_b = b_out(2, out_b)
    rounds(4, 8, wq_round)
    out_b = b_out(3, out_b)
    o_ref[:, DM:] = out_b.astype(BF16)
    rounds(8, 13, wq_round)
    w_wait(wo_v, SEM_WO)
    for h in range(H // 2):
        woh_s[h] = wo_v[:, h * DH:(h + 1) * DH]
    rounds(13, 18, wq_round)
    for h in range(H // 2, H):
        woh_s[h] = wo_v[:, h * DH:(h + 1) * DH]
    for j in range(LOOK - 2 * DELTA):
        kv_step(j, j % 2)

    w_wait(xa_v, SEM_XA)
    w_wait(wq_v, SEM_WQ)
    qa = jnp.dot(xa_v[...], wq_v[...], preferred_element_type=F32).astype(BF16)
    for h in range(H):
        qa_s[h] = qa[:, h * DH:(h + 1) * DH]

    row4 = jax.lax.broadcasted_iota(jnp.int32, (B, DH), 0)

    def scores(t):
        slot = t % NSLOT
        wait_all(kbuf.at[slot], kvsem.at[0, slot])
        s = jax.lax.dot_general(qa_s[t // B], kbuf[slot], NT,
                                preferred_element_type=F32) * SCALE
        p, l = _softmax_rows(s)
        p_s[t % PRING] = p.astype(BF16)
        l_s[t % PRING] = jnp.broadcast_to(l, (B, DH))

    def values(t, acc):
        slot = t % NSLOT
        wait_all(vbuf.at[slot], kvsem.at[1, slot])
        o = jnp.dot(p_s[t % PRING], vbuf[slot], preferred_element_type=F32) / l_s[t % PRING]
        o = jnp.where(row4 == t % B, o, 0.0).astype(BF16)
        return acc + jax.lax.dot_general(o, woh_s[t // B], NT, preferred_element_type=F32)

    def foreach(lo, hi, fn):
        def body(t, c):
            fn(t)
            return c
        jax.lax.fori_loop(lo, hi, body, 0)

    def steady(t, acc):
        kv_step(2 * t + LOOK, LOOK % 2)
        scores(t + DELTA)
        kv_step(2 * t + 1 + LOOK, (LOOK + 1) % 2)
        return jax.lax.cond(t >= 0, lambda: values(t, acc), lambda: acc)

    t_main = (NBLK - LOOK) // 2
    out_a = jax.lax.fori_loop(-DELTA, t_main, steady, jnp.zeros((B, DM), F32))
    tail_steps = range(2 * t_main + LOOK, NBLK + NS - 1)
    for j in tail_steps:
        kv_step(j, j % 2, 0)
    for j in tail_steps[:VSPLIT]:
        kv_step(j, j % 2, 1, tail_v=True)
    out_a = values(t_main, out_a)

    def tail_scores(t):
        scores(t)

        @pl.when(t == t_main + DELTA)
        def _():
            for j in tail_steps[VSPLIT:]:
                kv_step(j, j % 2, 1, tail_v=True)

    foreach(t_main + DELTA, NPAIR, tail_scores)
    out_a = jax.lax.fori_loop(t_main + 1, NPAIR, values, out_a)
    o_ref[:, :DM] = out_a.astype(BF16)


@jax.jit
def pallas_concat_heads__mha_block_cached__compressed_kv_cla__decode_kernel(
    A_x: jax.Array,
    A_k_cache: jax.Array,
    A_v_cache: jax.Array,
    A_wq: jax.Array,
    A_wo: jax.Array,
    B_x: jax.Array,
    B_c_kv: jax.Array,
    B_w_q: jax.Array,
    B_w_uk: jax.Array,
    B_w_uv: jax.Array,
    B_w_o: jax.Array,
):
    hbm = pl.BlockSpec(memory_space=pl.ANY)
    xa = A_x.reshape(B, DM)
    xb = B_x.reshape(B, DM)
    wo_t = A_wo.T
    wob_t = jnp.transpose(B_w_o, (0, 2, 1)).reshape(H * DM, DH)
    out = pl.pallas_call(
        _kernel,
        in_specs=[hbm] * 11,
        out_specs=pl.BlockSpec(memory_space=pltpu.VMEM),
        out_shape=jax.ShapeDtypeStruct((B, 2 * DM), BF16),
        scratch_shapes=[
            pltpu.VMEM((B, DM), BF16),
            pltpu.VMEM((B, DM), BF16),
            pltpu.VMEM((DM, HD), BF16),
            pltpu.VMEM((DM, HD), BF16),
            pltpu.VMEM((DM, H, DH), BF16),
            pltpu.VMEM((DC, H, DH), BF16),
            pltpu.VMEM((DC, H, DH), BF16),
            pltpu.VMEM((H * DM, DH), BF16),
            pltpu.VMEM((B, SK, DC), BF16),
            pltpu.VMEM((NSLOT, SK, DH), BF16),
            pltpu.VMEM((NSLOT, SK, DH), BF16),
            pltpu.VMEM((H, B, DH), BF16),
            pltpu.VMEM((H, DM, DH), BF16),
            pltpu.VMEM((PRING, B, SK), BF16),
            pltpu.VMEM((PRING, B, DH), F32),
            pltpu.VMEM((B * H, DC), F32),
            pltpu.VMEM((H, SK), BF16),
            pltpu.VMEM((H, DH), F32),
            pltpu.VMEM((B * H, DC), F32),
            pltpu.SemaphoreType.DMA((8 + B,)),
            pltpu.SemaphoreType.DMA((2, NSLOT)),
        ],
        compiler_params=pltpu.CompilerParams(vmem_limit_bytes=110 * 1024 * 1024,
                                             disable_bounds_checks=True,
                                             disable_semaphore_checks=True),
    )(xa, A_k_cache, A_v_cache, A_wq, wo_t, xb, B_c_kv, B_w_q, B_w_uk, B_w_uv, wob_t)
    return out.reshape(B, 1, 2 * DM)
```
